```python
import jax
import jax.numpy as jnp

def _softmax(x, axis=-1):
    return jax.nn.softmax(x, axis=axis)
def _gelu(x):
    return jax.nn.gelu(x, approximate=True)
def _silu(x):
    return jax.nn.silu(x)
def _sigmoid(x):
    return jax.nn.sigmoid(x)
def _layernorm(x, axis=-1, eps=1e-5):
    m = jnp.mean(x, axis=axis, keepdims=True)
    v = jnp.var(x, axis=axis, keepdims=True)
    return (x - m) / jnp.sqrt(v + eps)
def _scatter_add(tgt, idx, src, axis=0):
    return tgt.at[idx].add(src)
def _segment_sum(src, seg, n):
    return jax.ops.segment_sum(src, seg, n)
class _Rng:
    def __init__(self, key):
        self._k = key
    def _next(self):
        self._k, sub = jax.random.split(self._k)
        return sub
    def normal(self, shape):
        return jax.random.normal(self._next(), shape, dtype=jnp.bfloat16)
    def randint(self, lo, hi, shape):
        return jax.random.randint(self._next(), shape, lo, hi, dtype=jnp.int32)
    def uniform(self, shape, lo=0.0, hi=1.0):
        return jax.random.uniform(self._next(), shape, jnp.bfloat16, lo, hi)
    def permutation(self, n):
        return jax.random.permutation(self._next(), n)


kernel_name = 'concat_heads__mha_block_cached__compressed_kv_cla__decode'

def setup_inputs():
    _rng = _Rng(jax.random.key(int.from_bytes(__import__("os").urandom(4), "little")))
    _w = (lambda a: (lambda t: t.astype(jnp.bfloat16) if jnp.issubdtype(t.dtype, jnp.floating) else t)(jnp.asarray(a)))
    def _A_setup():
        B, Sq, D = 4, 1, 576
        H, Sk, Dh = 32, 4096, 128
        return {
            "x": _w((lambda *s: _rng.normal(s) * 0.05)(B, Sq, D)),
            "k_cache": _w((lambda *s: _rng.normal(s) * 0.05)(B, H, Sk, Dh)),
            "v_cache": _w((lambda *s: _rng.normal(s) * 0.05)(B, H, Sk, Dh)),
            "wq": _w((lambda *s: _rng.normal(s) * 0.05)(D, H * Dh) * (D ** -0.5)),
            "wo": _w((lambda *s: _rng.normal(s) * 0.05)(H * Dh, D) * ((H * Dh) ** -0.5)),
        }
    _A_in = _A_setup()

    def _B_setup():
        B, H, Sq, Sk, D, M = 4, 32, 1, 4096, 128, 576
        Dc = 4 * D
        return {
            "x": _w((lambda *s: _rng.normal(s) * 0.05)(B, Sq, M)),
            "c_kv": _w((lambda *s: _rng.normal(s) * 0.05)(B, Sk, Dc)),
            "w_q": _w((lambda *s: _rng.normal(s) * 0.05)(M, H, D) * (M ** -0.5)),
            "w_uk": _w((lambda *s: _rng.normal(s) * 0.05)(Dc, H, D) * (Dc ** -0.5)),
            "w_uv": _w((lambda *s: _rng.normal(s) * 0.05)(Dc, H, D) * (Dc ** -0.5)),
            "w_o": _w((lambda *s: _rng.normal(s) * 0.05)(H, D, M) * ((H * D) ** -0.5)),
        }
    _B_in = _B_setup()

    return {
        "A_x": _A_in["x"],
        "A_k_cache": _A_in["k_cache"],
        "A_v_cache": _A_in["v_cache"],
        "A_wq": _A_in["wq"],
        "A_wo": _A_in["wo"],
        "B_x": _B_in["x"],
        "B_c_kv": _B_in["c_kv"],
        "B_w_q": _B_in["w_q"],
        "B_w_uk": _B_in["w_uk"],
        "B_w_uv": _B_in["w_uv"],
        "B_w_o": _B_in["w_o"],
    }

def reference(A_x, A_k_cache, A_v_cache, A_wq, A_wo, B_x, B_c_kv, B_w_q, B_w_uk, B_w_uv, B_w_o):
    def _A_ref(x, k_cache, v_cache, wq, wo):
        B, Sq, D = x.shape
        H, Dh = 32, 128
        q = (lambda x, *d: x.transpose(*d))((x @ wq).reshape(B, Sq, H, Dh), 0, 2, 1, 3)
        scores = jnp.einsum("bhqd,bhkd->bhqk", q, k_cache) * (Dh ** -0.5)
        p = _softmax(scores, axis=-1)
        o = jnp.einsum("bhqk,bhkd->bhqd", p, v_cache)
        return (lambda x, *d: x.transpose(*d))(o, 0, 2, 1, 3).reshape(B, Sq, H * Dh) @ wo

    def _B_ref(x, c_kv, w_q, w_uk, w_uv, w_o):
        B, Sq, M = x.shape[0], x.shape[1], x.shape[2]
        Sk = c_kv.shape[1]
        H, D = w_q.shape[1], w_q.shape[2]
        q = jnp.einsum("bqm,mhd->bhqd", x, w_q)
        k = jnp.einsum("bkc,chd->bhkd", c_kv, w_uk)
        v = jnp.einsum("bkc,chd->bhkd", c_kv, w_uv)
        scores = jnp.einsum("bhqd,bhkd->bhqk", q, k) * (D ** -0.5)
        off = Sk - Sq
        qi = jnp.arange(Sq)[:, None]
        kj = jnp.arange(Sk)[None, :]
        cmask = kj <= (qi + off)
        scores = jnp.where(cmask[None, None], scores, -1e9)
        p = _softmax(scores, axis=-1)
        ctx = jnp.einsum("bhqk,bhkd->bhqd", p, v)
        return jnp.einsum("bhqd,hdm->bqm", ctx, w_o)

    a = _A_ref(A_x, A_k_cache, A_v_cache, A_wq, A_wo)
    b = _B_ref(B_x, B_c_kv, B_w_q, B_w_uk, B_w_uv, B_w_o)
    return jnp.concatenate([a, b], axis=-1)
```

```python
import jax
import jax.numpy as jnp
from jax import lax
import jax.experimental.pallas as pl
import jax.experimental.pallas.tpu as pltpu

_NT = (((1,), (1,)), ((), ()))
_NN = (((1,), (0,)), ((), ()))

_NBUF = 4


def _dot(a, b, dims):
    return lax.dot_general(a, b, dims, preferred_element_type=jnp.float32)


def _head_pair(w_ref, j, rows, n_heads):
    words = w_ref.bitcast(jnp.uint32)[pl.ds(j, rows, stride=n_heads // 2), :]
    even = pltpu.bitcast(words << 16, jnp.float32).astype(jnp.bfloat16)
    odd = pltpu.bitcast(words & jnp.uint32(0xFFFF0000), jnp.float32).astype(jnp.bfloat16)
    return even, odd


def _make_kernel(B, H, S, Dh, M, Dc):
    bf16, f32 = jnp.bfloat16, jnp.float32
    n_pairs = B * H
    n_cc = Dc // 128
    scale = Dh ** -0.5

    def kernel(xa_ref, xb_ref, k_hbm, v_hbm, awq_hbm, awo_hbm, ckv_hbm, bwq_hbm,
               wuk_hbm, wuv_hbm, bwo_hbm, out_ref,
               kbuf, vbuf, awq, awo, ckv, bwq, wuk, wuv, bwo,
               qa, oa, lat, kv_sem, w_sem):

        def kv_copies(i, slot):
            rows = pl.ds(pl.multiple_of(i * S, S), S)
            return (pltpu.make_async_copy(k_hbm.at[rows], kbuf.at[slot], kv_sem.at[0, slot]),
                    pltpu.make_async_copy(v_hbm.at[rows], vbuf.at[slot], kv_sem.at[1, slot]))

        pairs = ((awq_hbm, awq), (bwq_hbm, bwq), (wuk_hbm, wuk), (ckv_hbm, ckv),
                 (wuv_hbm, wuv), (bwo_hbm, bwo), (awo_hbm, awo))
        (c_awq, c_bwq, c_wuk, c_ckv, c_wuv, c_bwo, c_awo) = (
            pltpu.make_async_copy(s, d, w_sem.at[n]) for n, (s, d) in enumerate(pairs))

        for c in (c_awq, c_bwq, c_wuk, c_ckv, c_wuv, c_bwo, c_awo):
            c.start()
        for s in range(_NBUF):
            for c in kv_copies(s, s):
                c.start()

        def pad8(x_ref):
            x = x_ref[...].astype(f32)
            return jnp.concatenate([x, jnp.zeros((8 - B, M), f32)], axis=0).astype(bf16)

        xa, xb = pad8(xa_ref), pad8(xb_ref)

        c_awq.wait()
        for h in range(H):
            qa[h] = _dot(xa, awq[:, h * Dh:(h + 1) * Dh], _NN)

        c_bwq.wait()
        c_wuk.wait()

        def latent_q(j, carry):
            wq_pair = _head_pair(bwq, j, M, H)
            uk_pair = _head_pair(wuk, j, Dc, H)
            for e in range(2):
                q = _dot(xb, wq_pair[e], _NN).astype(bf16)
                ql = _dot(q, uk_pair[e], _NT)
                rows = pl.ds((2 * j + e) * 8, 8)
                for cc in range(n_cc):
                    lat[cc, rows, :] = ql[:, cc * 128:(cc + 1) * 128]
            return carry

        for j in range(H // 2):
            latent_q(j, 0)

        c_ckv.wait()

        def latent_attn(b, carry):
            rows = pl.ds(b, H, stride=8)
            ql = jnp.concatenate([lat[cc, rows, :] for cc in range(n_cc)], axis=1).astype(bf16)
            c = ckv[pl.ds(b * S, S), :]
            s = _dot(ql, c, _NT) * scale
            p = jnp.exp(s - jnp.max(s, axis=-1, keepdims=True))
            ctx = _dot(p.astype(bf16), c, _NN) / jnp.sum(p, axis=-1, keepdims=True)
            for cc in range(n_cc):
                lat[cc, rows, :] = ctx[:, cc * 128:(cc + 1) * 128]
            return carry

        for b in range(B):
            latent_attn(b, 0)

        c_wuv.wait()
        c_bwo.wait()

        def project_b(j, acc):
            uv_pair = _head_pair(wuv, j, Dc, H)
            for e in range(2):
                h = 2 * j + e
                rows = pl.ds(h * 8, 8)
                cl = jnp.concatenate([lat[cc, rows, :] for cc in range(n_cc)], axis=1).astype(bf16)
                ctx = _dot(cl, uv_pair[e], _NN).astype(bf16)
                acc = acc + _dot(ctx, bwo[pl.ds(h * M, M), :], _NT)
            return acc

        out_b = jnp.zeros((8, M), f32)
        for j in range(H // 2):
            out_b = project_b(j, out_b)

        oa[...] = jnp.zeros(oa.shape, f32)
        row_id = lax.broadcasted_iota(jnp.int32, (8, Dh), 0)

        def attend(i, carry):
            slot = i % _NBUF
            b, h = i // H, i % H
            ck, cv = kv_copies(i, slot)
            ck.wait()
            s = _dot(qa[h].astype(bf16), kbuf[slot], _NT) * scale
            p = jnp.exp(s - jnp.max(s, axis=-1, keepdims=True))
            cv.wait()
            o = _dot(p.astype(bf16), vbuf[slot], _NN) / jnp.sum(p, axis=-1, keepdims=True)
            oa[h] = jnp.where(row_id == b, o, oa[h])

            @pl.when(i + _NBUF < n_pairs)
            def _():
                for c in kv_copies(i + _NBUF, slot):
                    c.start()

            return carry

        lax.fori_loop(0, n_pairs, attend, 0)

        c_awo.wait()
        o_all = jnp.concatenate([oa[h] for h in range(H)], axis=1).astype(bf16)
        out_a = _dot(o_all, awo[...], _NT)
        out = jnp.concatenate([out_a, out_b], axis=1)
        out_ref[...] = out[:B].astype(out_ref.dtype)

    return kernel


@jax.jit
def pallas_concat_heads__mha_block_cached__compressed_kv_cla__decode_kernel(
    A_x: jax.Array,
    A_k_cache: jax.Array,
    A_v_cache: jax.Array,
    A_wq: jax.Array,
    A_wo: jax.Array,
    B_x: jax.Array,
    B_c_kv: jax.Array,
    B_w_q: jax.Array,
    B_w_uk: jax.Array,
    B_w_uv: jax.Array,
    B_w_o: jax.Array,
):
    B, H, S, Dh = A_k_cache.shape
    M = A_x.shape[-1]
    Dc = B_c_kv.shape[-1]
    bf16, f32 = jnp.bfloat16, jnp.float32

    in_vmem = pl.BlockSpec(memory_space=pltpu.VMEM)
    in_hbm = pl.BlockSpec(memory_space=pl.ANY)
    out = pl.pallas_call(
        _make_kernel(B, H, S, Dh, M, Dc),
        in_specs=[in_vmem, in_vmem] + [in_hbm] * 9,
        out_specs=in_vmem,
        out_shape=jax.ShapeDtypeStruct((B, 2 * M), A_x.dtype),
        scratch_shapes=[
            pltpu.VMEM((_NBUF, S, Dh), bf16),
            pltpu.VMEM((_NBUF, S, Dh), bf16),
            pltpu.VMEM((M, H * Dh), bf16),
            pltpu.VMEM((M, H * Dh), bf16),
            pltpu.VMEM((B * S, Dc), bf16),
            pltpu.VMEM((M * H, Dh), bf16),
            pltpu.VMEM((Dc * H, Dh), bf16),
            pltpu.VMEM((Dc * H, Dh), bf16),
            pltpu.VMEM((H * M, Dh), bf16),
            pltpu.VMEM((H, 8, Dh), f32),
            pltpu.VMEM((H, 8, Dh), f32),
            pltpu.VMEM((Dc // 128, H * 8, 128), f32),
            pltpu.SemaphoreType.DMA((2, _NBUF)),
            pltpu.SemaphoreType.DMA((7,)),
        ],
        compiler_params=pltpu.CompilerParams(vmem_limit_bytes=100 * 1024 * 1024),
    )(
        A_x.reshape(B, M),
        B_x.reshape(B, M),
        A_k_cache.reshape(B * H * S, Dh),
        A_v_cache.reshape(B * H * S, Dh),
        A_wq,
        A_wo.T,
        B_c_kv.reshape(B * S, Dc),
        B_w_q.reshape(M * H, Dh),
        B_w_uk.reshape(Dc * H, Dh),
        B_w_uv.reshape(Dc * H, Dh),
        B_w_o.transpose(0, 2, 1).reshape(H * M, Dh),
    )
    return out.reshape(B, 1, 2 * M)
```

```python
import jax
import jax.numpy as jnp
from jax import lax
import jax.experimental.pallas as pl
import jax.experimental.pallas.tpu as pltpu

_NT = (((1,), (1,)), ((), ()))
_NN = (((1,), (0,)), ((), ()))

_G = 8
_KC = 512
_NBUF = 3
_SEG = 64
_LC = 512
_CK = 1024


def _dot(a, b, dims):
    return lax.dot_general(a, b, dims, preferred_element_type=jnp.float32)


def _ds(index, size):
    return pl.ds(pl.multiple_of(index * size, size), size)


def _loop(lo, count, body):
    lax.fori_loop(lo, lo + count, lambda i, carry: (body(i), carry)[1], 0)


def _wait(buf, sem):
    pltpu.make_async_copy(buf, buf, sem).wait()


def _head_pair(w_ref, seg, j, n_heads):
    words = w_ref.bitcast(jnp.uint32)[seg, pl.ds(j, _SEG, stride=n_heads // 2), :]
    even = pltpu.bitcast(words << 16, jnp.float32).astype(jnp.bfloat16)
    odd = pltpu.bitcast(words & jnp.uint32(0xFFFF0000), jnp.float32).astype(jnp.bfloat16)
    return even, odd


def _softmax_step(first, carry, s, pv):
    m, l, acc = carry
    m = jnp.where(first, -jnp.inf, m)
    l = jnp.where(first, 0.0, l)
    acc = jnp.where(first, 0.0, acc)
    m_new = jnp.maximum(m, jnp.max(s, axis=-1, keepdims=True))
    alpha = jnp.exp(m - m_new)
    p = jnp.exp(s - m_new)
    l = alpha * l + jnp.sum(p, axis=-1, keepdims=True)
    acc = alpha * acc + pv(p.astype(jnp.bfloat16))
    return m_new, l, acc


def _softmax_init(rows, width):
    f32 = jnp.float32
    return jnp.zeros((rows, 1), f32), jnp.zeros((rows, 1), f32), jnp.zeros((rows, width), f32)


def _make_kernel(B, H, S, Dh, M, Dc):
    bf16, f32 = jnp.bfloat16, jnp.float32
    scale = Dh ** -0.5
    n_m, n_c = M // _SEG, Dc // _SEG
    n_cc = Dc // 128
    n_lc = H * Dh // _LC
    h_lc = _LC // Dh
    n_kc = S // _KC
    n_ck = S // _CK
    n_blocks = B * H // _G * n_kc

    def kernel(xa_hbm, xb_hbm, k_hbm, v_hbm, awq_hbm, awo_hbm, ckv_hbm, bwq_hbm,
               wuk_hbm, wuv_hbm, bwo_hbm, out_ref,
               xa_buf, xb_buf, kbuf, vbuf, awq, awo, ckv, bwq, wuk, wuv, bwo, xb_seg,
               by_head, by_batch, lat_head, lat_batch, k_sem, v_sem, awo_sem, sem):
        (xa_sem, xb_sem, bwq_sem, wuk_sem, ckv_sem, awq_sem, wuv_sem, bwo_sem) = (
            sem.at[n] for n in range(8))

        def halves(n):
            return ((pl.ds(0, n // 2), 0), (pl.ds(n // 2, n - n // 2), 1))

        def tall_piece(src, dst, dma_sem):
            def piece(t):
                rows = _ds(t, 32)
                for streams, priority in halves(src.shape[0]):
                    pltpu.make_async_copy(src.at[streams, rows], dst.at[streams, rows],
                                          dma_sem).start(priority=priority)
            return piece

        def wide_piece(src, dst, dma_sem, r, lc):
            rows = _ds(r, 8)
            for streams, priority in halves(n_m):
                pltpu.make_async_copy(src.at[streams, rows, _ds(lc, _LC)],
                                      dst.at[lc, streams, rows],
                                      dma_sem).start(priority=priority)

        def awq_piece(t):
            wide_piece(awq_hbm, awq, awq_sem, lax.div(t, n_lc), lax.rem(t, n_lc))

        def awo_piece(t):
            lc = lax.div(t, _SEG // 8)
            wide_piece(awo_hbm, awo, awo_sem.at[lc], lax.rem(t, _SEG // 8), lc)

        def ckv_piece(t):
            rows, half = _ds(t, 16), B * n_ck // 2
            for s in range(0, half, 2):
                for priority in range(2):
                    streams = pl.ds(priority * half + s, 2)
                    pltpu.make_async_copy(ckv_hbm.at[streams, rows], ckv.at[streams, rows],
                                          ckv_sem).start(priority=priority)

        kv_steps = _KC // 64

        def kv_piece(t):
            slot = lax.rem(lax.div(t, kv_steps), _NBUF)
            group = lax.div(t, kv_steps * n_kc)
            src_rows = _ds(lax.rem(t, kv_steps * n_kc), 64)
            dst_rows = _ds(lax.rem(t, kv_steps), 64)
            for s in range(0, _G, 2):
                heads = pl.ds(s, 2)
                pltpu.make_async_copy(k_hbm.at[group, heads, src_rows],
                                      kbuf.at[slot, heads, dst_rows],
                                      k_sem.at[slot]).start(priority=0)
                pltpu.make_async_copy(v_hbm.at[group, heads, src_rows],
                                      vbuf.at[slot, heads, dst_rows],
                                      v_sem.at[slot]).start(priority=1)

        bwq_piece = tall_piece(bwq_hbm, bwq, bwq_sem)
        wuk_piece = tall_piece(wuk_hbm, wuk, wuk_sem)
        wuv_piece = tall_piece(wuv_hbm, wuv, wuv_sem)
        bwo_piece = tall_piece(bwo_hbm, bwo, bwo_sem)

        _loop(0, 64, bwq_piece)
        x_copies = (pltpu.make_async_copy(xa_hbm, xa_buf, xa_sem),
                    pltpu.make_async_copy(xb_hbm, xb_buf, xb_sem))
        for c in x_copies:
            c.start()
        _loop(0, 64, wuk_piece)
        for c in x_copies:
            c.wait()

        def pad8(x_ref):
            return jnp.concatenate([x_ref[...].astype(f32), jnp.zeros((8 - B, M), f32)], axis=0)

        xb = pad8(xb_buf)
        for seg in range(n_m):
            xb_seg[seg] = xb[:, seg * _SEG:(seg + 1) * _SEG]
        by_head[...] = jnp.zeros(by_head.shape, f32)
        _wait(bwq, bwq_sem)

        def query_b(seg):
            x = xb_seg[seg].astype(bf16)
            for j in range(H // 2):
                for e, w in enumerate(_head_pair(bwq, seg, j, H)):
                    by_head[pl.ds((2 * j + e) * 8, 8), :] += _dot(x, w, _NN)
            _loop(seg * 4, 4, ckv_piece)

        _loop(0, n_m, query_b)

        def latent_tile(w_ref, cc, j):
            lo, hi = (_head_pair(w_ref, 2 * cc + i, j, H) for i in range(2))
            return [jnp.concatenate([lo[e], hi[e]], axis=0) for e in range(2)]

        _wait(wuk, wuk_sem)

        def latent_query(cc):
            for j in range(H // 2):
                for e, w in enumerate(latent_tile(wuk, cc, j)):
                    rows = pl.ds((2 * j + e) * 8, 8)
                    lat_head[cc, rows, :] = _dot(by_head[rows, :].astype(bf16), w, _NT)
            _loop(n_m * 4 + cc * 7, 7, ckv_piece)

        _loop(0, n_cc, latent_query)

        for b in range(B):
            for cc in range(n_cc):
                lat_batch[b, :, cc * 128:(cc + 1) * 128] = lat_head[cc, pl.ds(b, H, stride=8), :]

        _loop(0, 32, awq_piece)
        _wait(ckv, ckv_sem)

        def latent_attention(i, carry):
            b, chunk = lax.div(i, n_ck), lax.rem(i, n_ck)
            s = _dot(lat_batch[b].astype(bf16), ckv[i], _NT) * scale
            carry = _softmax_step(chunk == 0, carry, s, lambda p: _dot(p, ckv[i], _NN))

            @pl.when(chunk == n_ck - 1)
            def _():
                lat_batch[b] = carry[2] / carry[1]

            _loop(32 + i * 2, 2, awq_piece)
            _loop(i * 4, 4, wuv_piece)
            _loop(i * 4, 4, bwo_piece)
            return carry

        lax.fori_loop(0, B * n_ck, latent_attention, _softmax_init(H, Dc))

        for b in range(B):
            for cc in range(n_cc):
                lat_head[cc, pl.ds(b, H, stride=8), :] = lat_batch[b, :, cc * 128:(cc + 1) * 128]

        _loop(64, 8, bwo_piece)
        _loop(0, 4, kv_piece)
        by_head[...] = jnp.zeros(by_head.shape, f32)
        _wait(wuv, wuv_sem)

        def context_b(cc):
            for j in range(H // 2):
                for e, w in enumerate(latent_tile(wuv, cc, j)):
                    rows = pl.ds((2 * j + e) * 8, 8)
                    by_head[rows, :] += _dot(lat_head[cc, rows, :].astype(bf16), w, _NN)
            _loop(4 + cc * 3, 3, kv_piece)

        _loop(0, n_cc, context_b)
        _wait(bwo, bwo_sem)
        _wait(awq, awq_sem)
        xa = pad8(xa_buf).astype(bf16)

        def project_b_query_a(lc, out_b):
            q = _dot(xa, awq[lc].reshape(M, _LC), _NN)
            for t in range(h_lc):
                rows = _ds(lc * h_lc + t, 8)
                out_b += _dot(by_head[rows, :].astype(bf16), bwo[lc, pl.ds(t * M, M), :], _NT)
                by_head[rows, :] = q[:, t * Dh:(t + 1) * Dh]
            kv_piece(16 + lc)
            return out_b

        out_b = lax.fori_loop(0, n_lc, project_b_query_a, jnp.zeros((8, M), f32))
        out_ref[:, M:] = out_b[:B].astype(out_ref.dtype)

        for b in range(B):
            by_batch[pl.ds(b * H, H), :] = by_head[pl.ds(b, H, stride=8), :]

        def diagonal(parts):
            row = lax.broadcasted_iota(jnp.int32, parts[0].shape, 0)
            out = parts[0]
            for j in range(1, _G):
                out = jnp.where(row == j, parts[j], out)
            return out

        def attention(i, carry):
            slot = lax.rem(i, _NBUF)
            heads, chunk = _ds(lax.div(i, n_kc), _G), lax.rem(i, n_kc)
            _wait(kbuf.at[slot], k_sem.at[slot])
            _wait(vbuf.at[slot], v_sem.at[slot])
            q = by_batch[heads, :].astype(bf16)
            s = diagonal([_dot(q, kbuf[slot, j], _NT) for j in range(_G)]) * scale
            carry = _softmax_step(
                chunk == 0, carry, s,
                lambda p: diagonal([_dot(p, vbuf[slot, j], _NN) for j in range(_G)]))

            @pl.when(chunk == n_kc - 1)
            def _():
                by_batch[heads, :] = carry[2] / carry[1]

            @pl.when(i + _NBUF < n_blocks)
            def _():
                _loop((i + _NBUF) * kv_steps, kv_steps, kv_piece)

            @pl.when(i + _NBUF >= n_blocks)
            def _():
                n = i + _NBUF - n_blocks
                lo = lax.div(n * 64, _NBUF)
                _loop(lo, lax.div((n + 1) * 64, _NBUF) - lo, awo_piece)

            return carry

        lax.fori_loop(0, n_blocks, attention, _softmax_init(_G, Dh))

        for b in range(B):
            by_head[pl.ds(b, H, stride=8), :] = by_batch[pl.ds(b * H, H), :]

        def project_a(lc, out_a):
            o = jnp.concatenate([by_head[_ds(lc * h_lc + t, 8), :] for t in range(h_lc)], axis=1)
            _wait(awo.at[lc], awo_sem.at[lc])
            return out_a + _dot(o.astype(bf16), awo[lc].reshape(M, _LC), _NT)

        out_a = lax.fori_loop(0, n_lc, project_a, jnp.zeros((8, M), f32))
        out_ref[:, :M] = out_a[:B].astype(out_ref.dtype)

    return kernel


@jax.jit
def pallas_concat_heads__mha_block_cached__compressed_kv_cla__decode_kernel(
    A_x: jax.Array,
    A_k_cache: jax.Array,
    A_v_cache: jax.Array,
    A_wq: jax.Array,
    A_wo: jax.Array,
    B_x: jax.Array,
    B_c_kv: jax.Array,
    B_w_q: jax.Array,
    B_w_uk: jax.Array,
    B_w_uv: jax.Array,
    B_w_o: jax.Array,
):
    B, H, S, Dh = A_k_cache.shape
    M = A_x.shape[-1]
    Dc = B_c_kv.shape[-1]
    assert (B, H, S, Dh, M, Dc) == (4, 32, 4096, 128, 576, 512)
    bf16, f32 = jnp.bfloat16, jnp.float32
    n_m, n_c, n_lc = M // _SEG, Dc // _SEG, H * Dh // _LC

    out = pl.pallas_call(
        _make_kernel(B, H, S, Dh, M, Dc),
        in_specs=[pl.BlockSpec(memory_space=pl.ANY)] * 11,
        out_specs=pl.BlockSpec(memory_space=pltpu.VMEM),
        out_shape=jax.ShapeDtypeStruct((B, 2 * M), A_x.dtype),
        scratch_shapes=[
            pltpu.VMEM((B, M), bf16),
            pltpu.VMEM((B, M), bf16),
            pltpu.VMEM((_NBUF, _G, _KC, Dh), bf16),
            pltpu.VMEM((_NBUF, _G, _KC, Dh), bf16),
            pltpu.VMEM((n_lc, n_m, _SEG, _LC), bf16),
            pltpu.VMEM((n_lc, n_m, _SEG, _LC), bf16),
            pltpu.VMEM((B * S // _CK, _CK, Dc), bf16),
            pltpu.VMEM((n_m, _SEG * H, Dh), bf16),
            pltpu.VMEM((n_c, _SEG * H, Dh), bf16),
            pltpu.VMEM((n_c, _SEG * H, Dh), bf16),
            pltpu.VMEM((n_lc, H * M // n_lc, Dh), bf16),
            pltpu.VMEM((n_m, 8, _SEG), f32),
            pltpu.VMEM((H * 8, Dh), f32),
            pltpu.VMEM((B * H, Dh), f32),
            pltpu.VMEM((Dc // 128, H * 8, 128), f32),
            pltpu.VMEM((B, H, Dc), f32),
            pltpu.SemaphoreType.DMA((_NBUF,)),
            pltpu.SemaphoreType.DMA((_NBUF,)),
            pltpu.SemaphoreType.DMA((n_lc,)),
            pltpu.SemaphoreType.DMA((8,)),
        ],
        compiler_params=pltpu.CompilerParams(
            vmem_limit_bytes=80 * 1024 * 1024, disable_bounds_checks=True),
    )(
        A_x.reshape(B, M),
        B_x.reshape(B, M),
        A_k_cache.reshape(B * H // _G, _G, S, Dh),
        A_v_cache.reshape(B * H // _G, _G, S, Dh),
        A_wq.reshape(n_m, _SEG, H * Dh),
        A_wo.T.reshape(n_m, _SEG, H * Dh),
        B_c_kv.reshape(B * S // _CK, _CK, Dc),
        B_w_q.reshape(n_m, _SEG * H, Dh),
        B_w_uk.reshape(n_c, _SEG * H, Dh),
        B_w_uv.reshape(n_c, _SEG * H, Dh),
        B_w_o.transpose(0, 2, 1).reshape(n_lc, H * M // n_lc, Dh),
    )
    return out.reshape(B, 1, 2 * M)
```

```python
import jax
import jax.numpy as jnp
from jax import lax
import jax.experimental.pallas as pl
import jax.experimental.pallas.tpu as pltpu

_NT = (((1,), (1,)), ((), ()))
_NN = (((1,), (0,)), ((), ()))

_G = 8
_KC = 512
_NBUF = 5
_SEG = 64
_LC = 512
_CK = 1024


def _dot(a, b, dims):
    return lax.dot_general(a, b, dims, preferred_element_type=jnp.float32)


def _ds(index, size):
    return pl.ds(pl.multiple_of(index * size, size), size)


def _loop(lo, count, body):
    lax.fori_loop(lo, lo + count, lambda i, carry: (body(i), carry)[1], 0)


def _wait(buf, sem):
    pltpu.make_async_copy(buf, buf, sem).wait()


def _head_pair(w_ref, seg, j, n_heads):
    words = w_ref.bitcast(jnp.uint32)[seg, pl.ds(j, _SEG, stride=n_heads // 2), :]
    even = pltpu.bitcast(words << 16, jnp.float32).astype(jnp.bfloat16)
    odd = pltpu.bitcast(words & jnp.uint32(0xFFFF0000), jnp.float32).astype(jnp.bfloat16)
    return even, odd


def _softmax_step(first, carry, s, pv):
    m, l, acc = carry
    m = jnp.where(first, -jnp.inf, m)
    l = jnp.where(first, 0.0, l)
    acc = jnp.where(first, 0.0, acc)
    m_new = jnp.maximum(m, jnp.max(s, axis=-1, keepdims=True))
    alpha = jnp.exp(m - m_new)
    p = jnp.exp(s - m_new)
    l = alpha * l + jnp.sum(p, axis=-1, keepdims=True)
    acc = alpha * acc + pv(p.astype(jnp.bfloat16))
    return m_new, l, acc


def _softmax_init(rows, width):
    f32 = jnp.float32
    return jnp.zeros((rows, 1), f32), jnp.zeros((rows, 1), f32), jnp.zeros((rows, width), f32)


def _make_kernel(B, H, S, Dh, M, Dc):
    bf16, f32 = jnp.bfloat16, jnp.float32
    scale = Dh ** -0.5
    n_m, n_c = M // _SEG, Dc // _SEG
    n_cc = Dc // 128
    n_lc = H * Dh // _LC
    h_lc = _LC // Dh
    n_kc = S // _KC
    n_ck = S // _CK
    n_blocks = B * H // _G * n_kc

    def kernel(xa_hbm, xb_hbm, k_hbm, v_hbm, awq_hbm, awo_hbm, ckv_hbm, bwq_hbm,
               wuk_hbm, wuv_hbm, bwo_hbm, out_ref,
               xa_buf, xb_buf, kbuf, vbuf, awq, awo, ckv, bwq, wuk, wuv, bwo, xb_seg,
               by_head, by_batch, lat_head, lat_batch, k_sem, v_sem, awo_sem, sem):
        (xa_sem, xb_sem, bwq_sem, wuk_sem, ckv_sem, awq_sem, wuv_sem, bwo_sem) = (
            sem.at[n] for n in range(8))

        def halves(n):
            return ((pl.ds(0, n // 2), 0), (pl.ds(n // 2, n - n // 2), 1))

        def tall_piece(src, dst, dma_sem):
            def piece(t):
                rows = _ds(t, 32)
                for streams, priority in halves(src.shape[0]):
                    pltpu.make_async_copy(src.at[streams, rows], dst.at[streams, rows],
                                          dma_sem).start(priority=priority)
            return piece

        def wide_piece(src, dst, dma_sem, r, lc):
            rows = _ds(r, 8)
            for streams, priority in halves(n_m):
                pltpu.make_async_copy(src.at[streams, rows, _ds(lc, _LC)],
                                      dst.at[lc, streams, rows],
                                      dma_sem).start(priority=priority)

        def awq_piece(t):
            wide_piece(awq_hbm, awq, awq_sem, lax.div(t, n_lc), lax.rem(t, n_lc))

        def awo_piece(t):
            lc = lax.div(t, _SEG // 8)
            wide_piece(awo_hbm, awo, awo_sem.at[lc], lax.rem(t, _SEG // 8), lc)

        def ckv_piece(t):
            rows, half = _ds(t, 16), B * n_ck // 2
            for s in range(0, half, 2):
                for priority in range(2):
                    streams = pl.ds(priority * half + s, 2)
                    pltpu.make_async_copy(ckv_hbm.at[streams, rows], ckv.at[streams, rows],
                                          ckv_sem).start(priority=priority)

        kv_steps = _KC // 64

        def kv_piece(t):
            slot = lax.rem(lax.div(t, kv_steps), _NBUF)
            group = lax.div(t, kv_steps * n_kc)
            src_rows = _ds(lax.rem(t, kv_steps * n_kc), 64)
            dst_rows = _ds(lax.rem(t, kv_steps), 64)
            for s in range(0, _G, 2):
                heads = pl.ds(s, 2)
                pltpu.make_async_copy(k_hbm.at[group, heads, src_rows],
                                      kbuf.at[slot, heads, dst_rows],
                                      k_sem.at[slot]).start(priority=0)
                pltpu.make_async_copy(v_hbm.at[group, heads, src_rows],
                                      vbuf.at[slot, heads, dst_rows],
                                      v_sem.at[slot]).start(priority=1)

        bwq_piece = tall_piece(bwq_hbm, bwq, bwq_sem)
        wuk_piece = tall_piece(wuk_hbm, wuk, wuk_sem)
        wuv_piece = tall_piece(wuv_hbm, wuv, wuv_sem)
        bwo_piece = tall_piece(bwo_hbm, bwo, bwo_sem)

        _loop(0, 64, bwq_piece)
        x_copies = (pltpu.make_async_copy(xa_hbm, xa_buf, xa_sem),
                    pltpu.make_async_copy(xb_hbm, xb_buf, xb_sem))
        for c in x_copies:
            c.start()
        _loop(0, 64, wuk_piece)
        for c in x_copies:
            c.wait()

        def pad8(x_ref):
            return jnp.concatenate([x_ref[...].astype(f32), jnp.zeros((8 - B, M), f32)], axis=0)

        xb = pad8(xb_buf)
        for seg in range(n_m):
            xb_seg[seg] = xb[:, seg * _SEG:(seg + 1) * _SEG]
        by_head[...] = jnp.zeros(by_head.shape, f32)
        _wait(bwq, bwq_sem)

        def query_b(seg):
            x = xb_seg[seg].astype(bf16)
            for j in range(H // 2):
                for e, w in enumerate(_head_pair(bwq, seg, j, H)):
                    by_head[pl.ds((2 * j + e) * 8, 8), :] += _dot(x, w, _NN)
            _loop(seg * 4, 4, ckv_piece)

        _loop(0, n_m, query_b)

        def latent_tile(w_ref, cc, j):
            lo, hi = (_head_pair(w_ref, 2 * cc + i, j, H) for i in range(2))
            return [jnp.concatenate([lo[e], hi[e]], axis=0) for e in range(2)]

        _wait(wuk, wuk_sem)

        def latent_query(cc):
            for j in range(H // 2):
                for e, w in enumerate(latent_tile(wuk, cc, j)):
                    rows = pl.ds((2 * j + e) * 8, 8)
                    lat_head[cc, rows, :] = _dot(by_head[rows, :].astype(bf16), w, _NT)
            _loop(n_m * 4 + cc * 7, 7, ckv_piece)

        _loop(0, n_cc, latent_query)

        for b in range(B):
            for cc in range(n_cc):
                lat_batch[b, :, cc * 128:(cc + 1) * 128] = lat_head[cc, pl.ds(b, H, stride=8), :]

        _loop(0, 32, awq_piece)
        _wait(ckv, ckv_sem)

        def latent_attention(i, carry):
            b, chunk = lax.div(i, n_ck), lax.rem(i, n_ck)
            s = _dot(lat_batch[b].astype(bf16), ckv[i], _NT) * scale
            carry = _softmax_step(chunk == 0, carry, s, lambda p: _dot(p, ckv[i], _NN))

            @pl.when(chunk == n_ck - 1)
            def _():
                lat_batch[b] = carry[2] / carry[1]

            _loop(32 + i * 2, 2, awq_piece)
            _loop(i * 4, 4, wuv_piece)
            _loop(i * 4, 4, bwo_piece)
            kv_piece(i)
            return carry

        lax.fori_loop(0, B * n_ck, latent_attention, _softmax_init(H, Dc))

        for b in range(B):
            for cc in range(n_cc):
                lat_head[cc, pl.ds(b, H, stride=8), :] = lat_batch[b, :, cc * 128:(cc + 1) * 128]

        _loop(64, 8, bwo_piece)
        _loop(16, 4, kv_piece)
        by_head[...] = jnp.zeros(by_head.shape, f32)
        _wait(wuv, wuv_sem)

        def context_b(cc):
            for j in range(H // 2):
                for e, w in enumerate(latent_tile(wuv, cc, j)):
                    rows = pl.ds((2 * j + e) * 8, 8)
                    by_head[rows, :] += _dot(lat_head[cc, rows, :].astype(bf16), w, _NN)
            _loop(20 + cc * 3, 3, kv_piece)

        _loop(0, n_cc, context_b)
        _wait(bwo, bwo_sem)
        _wait(awq, awq_sem)
        xa = pad8(xa_buf).astype(bf16)

        def project_b_query_a(lc, out_b):
            q = _dot(xa, awq[lc].reshape(M, _LC), _NN)
            for t in range(h_lc):
                rows = _ds(lc * h_lc + t, 8)
                out_b += _dot(by_head[rows, :].astype(bf16), bwo[lc, pl.ds(t * M, M), :], _NT)
                by_head[rows, :] = q[:, t * Dh:(t + 1) * Dh]
            kv_piece(32 + lc)
            return out_b

        out_b = lax.fori_loop(0, n_lc, project_b_query_a, jnp.zeros((8, M), f32))
        out_ref[:, M:] = out_b[:B].astype(out_ref.dtype)

        for b in range(B):
            by_batch[pl.ds(b * H, H), :] = by_head[pl.ds(b, H, stride=8), :]

        def diagonal(parts):
            row = lax.broadcasted_iota(jnp.int32, parts[0].shape, 0)
            out = parts[0]
            for j in range(1, _G):
                out = jnp.where(row == j, parts[j], out)
            return out

        def attention(i, carry):
            slot = lax.rem(i, _NBUF)
            heads, chunk = _ds(lax.div(i, n_kc), _G), lax.rem(i, n_kc)
            _wait(kbuf.at[slot], k_sem.at[slot])
            _wait(vbuf.at[slot], v_sem.at[slot])
            q = by_batch[heads, :].astype(bf16)
            s = diagonal([_dot(q, kbuf[slot, j], _NT) for j in range(_G)]) * scale
            carry = _softmax_step(
                chunk == 0, carry, s,
                lambda p: diagonal([_dot(p, vbuf[slot, j], _NN) for j in range(_G)]))

            @pl.when(chunk == n_kc - 1)
            def _():
                by_batch[heads, :] = carry[2] / carry[1]

            @pl.when(i + _NBUF < n_blocks)
            def _():
                _loop((i + _NBUF) * kv_steps, kv_steps, kv_piece)

            @pl.when(i + _NBUF >= n_blocks)
            def _():
                n = i + _NBUF - n_blocks
                lo = lax.div(n * 64, _NBUF)
                _loop(lo, lax.div((n + 1) * 64, _NBUF) - lo, awo_piece)

            return carry

        lax.fori_loop(0, n_blocks, attention, _softmax_init(_G, Dh))

        for b in range(B):
            by_head[pl.ds(b, H, stride=8), :] = by_batch[pl.ds(b * H, H), :]

        def project_a(lc, out_a):
            o = jnp.concatenate([by_head[_ds(lc * h_lc + t, 8), :] for t in range(h_lc)], axis=1)
            _wait(awo.at[lc], awo_sem.at[lc])
            return out_a + _dot(o.astype(bf16), awo[lc].reshape(M, _LC), _NT)

        out_a = lax.fori_loop(0, n_lc, project_a, jnp.zeros((8, M), f32))
        out_ref[:, :M] = out_a[:B].astype(out_ref.dtype)

    return kernel


@jax.jit
def pallas_concat_heads__mha_block_cached__compressed_kv_cla__decode_kernel(
    A_x: jax.Array,
    A_k_cache: jax.Array,
    A_v_cache: jax.Array,
    A_wq: jax.Array,
    A_wo: jax.Array,
    B_x: jax.Array,
    B_c_kv: jax.Array,
    B_w_q: jax.Array,
    B_w_uk: jax.Array,
    B_w_uv: jax.Array,
    B_w_o: jax.Array,
):
    B, H, S, Dh = A_k_cache.shape
    M = A_x.shape[-1]
    Dc = B_c_kv.shape[-1]
    assert (B, H, S, Dh, M, Dc) == (4, 32, 4096, 128, 576, 512)
    bf16, f32 = jnp.bfloat16, jnp.float32
    n_m, n_c, n_lc = M // _SEG, Dc // _SEG, H * Dh // _LC

    out = pl.pallas_call(
        _make_kernel(B, H, S, Dh, M, Dc),
        in_specs=[pl.BlockSpec(memory_space=pl.ANY)] * 11,
        out_specs=pl.BlockSpec(memory_space=pltpu.VMEM),
        out_shape=jax.ShapeDtypeStruct((B, 2 * M), A_x.dtype),
        scratch_shapes=[
            pltpu.VMEM((B, M), bf16),
            pltpu.VMEM((B, M), bf16),
            pltpu.VMEM((_NBUF, _G, _KC, Dh), bf16),
            pltpu.VMEM((_NBUF, _G, _KC, Dh), bf16),
            pltpu.VMEM((n_lc, n_m, _SEG, _LC), bf16),
            pltpu.VMEM((n_lc, n_m, _SEG, _LC), bf16),
            pltpu.VMEM((B * S // _CK, _CK, Dc), bf16),
            pltpu.VMEM((n_m, _SEG * H, Dh), bf16),
            pltpu.VMEM((n_c, _SEG * H, Dh), bf16),
            pltpu.VMEM((n_c, _SEG * H, Dh), bf16),
            pltpu.VMEM((n_lc, H * M // n_lc, Dh), bf16),
            pltpu.VMEM((n_m, 8, _SEG), f32),
            pltpu.VMEM((H * 8, Dh), f32),
            pltpu.VMEM((B * H, Dh), f32),
            pltpu.VMEM((Dc // 128, H * 8, 128), f32),
            pltpu.VMEM((B, H, Dc), f32),
            pltpu.SemaphoreType.DMA((_NBUF,)),
            pltpu.SemaphoreType.DMA((_NBUF,)),
            pltpu.SemaphoreType.DMA((n_lc,)),
            pltpu.SemaphoreType.DMA((8,)),
        ],
        compiler_params=pltpu.CompilerParams(
            vmem_limit_bytes=80 * 1024 * 1024, disable_bounds_checks=True),
    )(
        A_x.reshape(B, M),
        B_x.reshape(B, M),
        A_k_cache.reshape(B * H // _G, _G, S, Dh),
        A_v_cache.reshape(B * H // _G, _G, S, Dh),
        A_wq.reshape(n_m, _SEG, H * Dh),
        A_wo.T.reshape(n_m, _SEG, H * Dh),
        B_c_kv.reshape(B * S // _CK, _CK, Dc),
        B_w_q.reshape(n_m, _SEG * H, Dh),
        B_w_uk.reshape(n_c, _SEG * H, Dh),
        B_w_uv.reshape(n_c, _SEG * H, Dh),
        B_w_o.transpose(0, 2, 1).reshape(n_lc, H * M // n_lc, Dh),
    )
    return out.reshape(B, 1, 2 * M)
```

```python
import jax
import jax.numpy as jnp
from jax import lax
import jax.experimental.pallas as pl
import jax.experimental.pallas.tpu as pltpu

_NT = (((1,), (1,)), ((), ()))
_NN = (((1,), (0,)), ((), ()))

_G = 8
_KC = 512
_NBUF = 4
_SEG = 64
_LC = 512
_CK = 1024


def _dot(a, b, dims):
    return lax.dot_general(a, b, dims, preferred_element_type=jnp.float32)


def _ds(index, size):
    return pl.ds(pl.multiple_of(index * size, size), size)


def _loop(lo, count, body):
    lax.fori_loop(lo, lo + count, lambda i, carry: (body(i), carry)[1], 0)


def _share(n, parts, total, body):
    lo = lax.div(n * total, parts)
    _loop(lo, lax.div((n + 1) * total, parts) - lo, body)


def _wait(buf, sem):
    pltpu.make_async_copy(buf, buf, sem).wait()


def _head_pair(w_ref, seg, j, n_heads):
    words = w_ref.bitcast(jnp.uint32)[seg, pl.ds(j, _SEG, stride=n_heads // 2), :]
    even = pltpu.bitcast(words << 16, jnp.float32).astype(jnp.bfloat16)
    odd = pltpu.bitcast(words & jnp.uint32(0xFFFF0000), jnp.float32).astype(jnp.bfloat16)
    return even, odd


def _softmax_step(carry, s, pv):
    m, l, acc = carry
    m_new = jnp.maximum(m, jnp.max(s, axis=-1, keepdims=True))
    alpha = jnp.exp(m - m_new)
    p = jnp.exp(s - m_new)
    l = alpha * l + jnp.sum(p, axis=-1, keepdims=True)
    acc = alpha * acc + pv(p.astype(jnp.bfloat16))
    return m_new, l, acc


def _softmax_init(rows, width):
    f32 = jnp.float32
    return jnp.zeros((rows, 1), f32), jnp.zeros((rows, 1), f32), jnp.zeros((rows, width), f32)


def _make_kernel(B, H, S, Dh, M, Dc):
    bf16, f32 = jnp.bfloat16, jnp.float32
    scale = Dh ** -0.5
    n_m, n_c = M // _SEG, Dc // _SEG
    n_cc = Dc // 128
    n_lc = H * Dh // _LC
    h_lc = _LC // Dh
    n_kc = S // _KC
    n_ck = S // _CK
    n_blocks = B * H // _G * n_kc

    def body(xa_hbm, xb_hbm, k_hbm, v_hbm, awq_hbm, awo_hbm, ckv_hbm, bwq_hbm,
               wuk_hbm, wuv_hbm, bwo_hbm, out_ref,
               xa_buf, xb_buf, kbuf, vbuf, awq, awo, ckv, bwq, wuk, wuv, bwo, xb_seg,
               by_head, by_batch, lat_head, lat_batch, lat_m, lat_l, lat_acc, k_sem, v_sem, awo_sem, ckv_sem, sem):
        xa_sem, xb_sem, bwq_sem, wuk_sem, awq_sem, wuv_sem, bwo_sem = (
            sem.at[n] for n in range(7))

        def halves(n):
            return ((pl.ds(0, n // 2), 0), (pl.ds(n // 2, n - n // 2), 1))

        def tall_piece(src, dst, dma_sem):
            def piece(t):
                rows = _ds(t, 32)
                for streams, priority in halves(src.shape[0]):
                    pltpu.make_async_copy(src.at[streams, rows], dst.at[streams, rows],
                                          dma_sem).start(priority=priority)
            return piece

        def wide_piece(src, dst, dma_sem, r, lc):
            rows = _ds(r, 8)
            for streams, priority in halves(n_m):
                pltpu.make_async_copy(src.at[streams, rows, _ds(lc, _LC)],
                                      dst.at[lc, streams, rows],
                                      dma_sem).start(priority=priority)

        def awq_piece(t):
            wide_piece(awq_hbm, awq, awq_sem, lax.div(t, n_lc), lax.rem(t, n_lc))

        def awo_piece(t):
            lc = lax.div(t, _SEG // 8)
            wide_piece(awo_hbm, awo, awo_sem.at[lc], lax.rem(t, _SEG // 8), lc)

        def ckv_piece(t):
            steps = _CK // n_ck // 16
            chunk, rows = lax.div(t, steps), _ds(lax.rem(t, steps), 16)
            for b in range(B // 2):
                for s in range(0, n_ck, 2):
                    for priority in range(2):
                        batch, streams = b + priority * B // 2, pl.ds(s, 2)
                        pltpu.make_async_copy(ckv_hbm.at[batch, streams, _ds(t, 16)],
                                              ckv.at[chunk, batch, streams, rows],
                                              ckv_sem.at[chunk]).start(priority=priority)

        kv_steps = _KC // 64

        def kv_piece(t):
            slot = lax.rem(lax.div(t, kv_steps), _NBUF)
            group = lax.div(t, kv_steps * n_kc)
            src_rows = _ds(lax.rem(t, kv_steps * n_kc), 64)
            dst_rows = _ds(lax.rem(t, kv_steps), 64)
            for s in range(0, _G, 2):
                heads = pl.ds(s, 2)
                pltpu.make_async_copy(k_hbm.at[group, heads, src_rows],
                                      kbuf.at[slot, heads, dst_rows],
                                      k_sem.at[slot]).start(priority=0)
                pltpu.make_async_copy(v_hbm.at[group, heads, src_rows],
                                      vbuf.at[slot, heads, dst_rows],
                                      v_sem.at[slot]).start(priority=1)

        bwq_piece = tall_piece(bwq_hbm, bwq, bwq_sem)
        wuk_piece = tall_piece(wuk_hbm, wuk, wuk_sem)
        wuv_piece = tall_piece(wuv_hbm, wuv, wuv_sem)
        bwo_piece = tall_piece(bwo_hbm, bwo, bwo_sem)

        _loop(0, 64, bwq_piece)
        x_copies = (pltpu.make_async_copy(xa_hbm, xa_buf, xa_sem),
                    pltpu.make_async_copy(xb_hbm, xb_buf, xb_sem))
        for c in x_copies:
            c.start()
        _loop(0, 64, wuk_piece)
        for c in x_copies:
            c.wait()

        def pad8(x_ref):
            return jnp.concatenate([x_ref[...].astype(f32), jnp.zeros((8 - B, M), f32)], axis=0)

        xb = pad8(xb_buf)
        for seg in range(n_m):
            xb_seg[seg] = xb[:, seg * _SEG:(seg + 1) * _SEG]
        by_head[...] = jnp.zeros(by_head.shape, f32)
        _wait(bwq, bwq_sem)

        def query_b(seg):
            x = xb_seg[seg].astype(bf16)
            for j in range(H // 2):
                for e, w in enumerate(_head_pair(bwq, seg, j, H)):
                    by_head[pl.ds((2 * j + e) * 8, 8), :] += _dot(x, w, _NN)
            _loop(seg * 2, 2, ckv_piece)

        _loop(0, n_m, query_b)

        def latent_tile(w_ref, cc, j):
            lo, hi = (_head_pair(w_ref, 2 * cc + i, j, H) for i in range(2))
            return [jnp.concatenate([lo[e], hi[e]], axis=0) for e in range(2)]

        _wait(wuk, wuk_sem)

        def latent_query(cc):
            for j in range(H // 2):
                for e, w in enumerate(latent_tile(wuk, cc, j)):
                    rows = pl.ds((2 * j + e) * 8, 8)
                    lat_head[cc, rows, :] = _dot(by_head[rows, :].astype(bf16), w, _NT)
            _loop(18 + cc * 4, 4, ckv_piece)

        _loop(0, n_cc, latent_query)

        for b in range(B):
            for cc in range(n_cc):
                lat_batch[b, :, cc * 128:(cc + 1) * 128] = lat_head[cc, pl.ds(b, H, stride=8), :]

        lat_m[...] = jnp.full(lat_m.shape, -jnp.inf, f32)
        lat_l[...] = jnp.zeros(lat_l.shape, f32)
        lat_acc[...] = jnp.zeros(lat_acc.shape, f32)

        def latent_attention(i):
            chunk, b = lax.div(i, B), lax.rem(i, B)

            @pl.when(b == 0)
            def _():
                _wait(ckv.at[chunk], ckv_sem.at[chunk])

            def cache():
                return ckv[chunk, b].reshape(S // n_ck, Dc)

            s = _dot(lat_batch[b].astype(bf16), cache(), _NT) * scale
            lat_m[b], lat_l[b], lat_acc[b] = _softmax_step(
                (lat_m[b], lat_l[b], lat_acc[b]), s, lambda p: _dot(p, cache(), _NN))

            @pl.when(i < 6)
            def _():
                _loop(34 + i * 5, 5, ckv_piece)

            @pl.when(i >= 6)
            def _():
                for piece, total in ((wuv_piece, 64), (awq_piece, 64), (bwo_piece, 72)):
                    _share(i - 6, B * n_ck - 6, total, piece)

        _loop(0, B * n_ck, latent_attention)

        for b in range(B):
            ctx = lat_acc[b] / lat_l[b]
            for cc in range(n_cc):
                lat_head[cc, pl.ds(b, H, stride=8), :] = ctx[:, cc * 128:(cc + 1) * 128]

        _loop(0, 8, kv_piece)
        by_head[...] = jnp.zeros(by_head.shape, f32)
        _wait(wuv, wuv_sem)

        def context_b(cc):
            for j in range(H // 2):
                for e, w in enumerate(latent_tile(wuv, cc, j)):
                    rows = pl.ds((2 * j + e) * 8, 8)
                    by_head[rows, :] += _dot(lat_head[cc, rows, :].astype(bf16), w, _NN)
            _loop(8 + cc * 4, 4, kv_piece)

        _loop(0, n_cc, context_b)
        _wait(bwo, bwo_sem)
        _wait(awq, awq_sem)
        xa = pad8(xa_buf).astype(bf16)

        def project_b_query_a(lc, out_b):
            q = _dot(xa, awq[lc].reshape(M, _LC), _NN)
            for t in range(h_lc):
                rows = _ds(lc * h_lc + t, 8)
                out_b += _dot(by_head[rows, :].astype(bf16), bwo[lc, pl.ds(t * M, M), :], _NT)
                by_head[rows, :] = q[:, t * Dh:(t + 1) * Dh]
            kv_piece(24 + lc)
            return out_b

        out_b = lax.fori_loop(0, n_lc, project_b_query_a, jnp.zeros((8, M), f32))
        out_ref[:, M:] = out_b[:B].astype(out_ref.dtype)

        for b in range(B):
            by_batch[pl.ds(b * H, H), :] = by_head[pl.ds(b, H, stride=8), :]

        def diagonal(parts):
            row = lax.broadcasted_iota(jnp.int32, parts[0].shape, 0)
            out = parts[0]
            for j in range(1, _G):
                out = jnp.where(row == j, parts[j], out)
            return out

        def attention(i, carry):
            slot = lax.rem(i, _NBUF)
            heads, chunk = _ds(lax.div(i, n_kc), _G), lax.rem(i, n_kc)
            _wait(kbuf.at[slot], k_sem.at[slot])
            _wait(vbuf.at[slot], v_sem.at[slot])
            q = by_batch[heads, :].astype(bf16)
            s = diagonal([_dot(q, kbuf[slot, j], _NT) for j in range(_G)]) * scale
            carry = tuple(jnp.where(chunk == 0, fill, c)
                          for fill, c in zip((-jnp.inf, 0.0, 0.0), carry))
            carry = _softmax_step(
                carry, s,
                lambda p: diagonal([_dot(p, vbuf[slot, j], _NN) for j in range(_G)]))

            @pl.when(chunk == n_kc - 1)
            def _():
                by_batch[heads, :] = carry[2] / carry[1]

            @pl.when(i + _NBUF < n_blocks)
            def _():
                _loop((i + _NBUF) * kv_steps, kv_steps, kv_piece)

            @pl.when(i + _NBUF >= n_blocks)
            def _():
                _share(i + _NBUF - n_blocks, _NBUF, 64, awo_piece)

            return carry

        lax.fori_loop(0, n_blocks, attention, _softmax_init(_G, Dh))

        for b in range(B):
            by_head[pl.ds(b, H, stride=8), :] = by_batch[pl.ds(b * H, H), :]

        def project_a(lc, out_a):
            o = jnp.concatenate([by_head[_ds(lc * h_lc + t, 8), :] for t in range(h_lc)], axis=1)
            _wait(awo.at[lc], awo_sem.at[lc])
            return out_a + _dot(o.astype(bf16), awo[lc].reshape(M, _LC), _NT)

        out_a = lax.fori_loop(0, n_lc, project_a, jnp.zeros((8, M), f32))
        out_ref[:, :M] = out_a[:B].astype(out_ref.dtype)

    def kernel(*refs):
        sizes = (_NBUF, _NBUF, n_lc, n_ck, 7)
        pl.run_scoped(lambda *sems: body(*refs, *sems),
                      *(pltpu.SemaphoreType.DMA((n,)) for n in sizes))

    return kernel


@jax.jit
def pallas_concat_heads__mha_block_cached__compressed_kv_cla__decode_kernel(
    A_x: jax.Array,
    A_k_cache: jax.Array,
    A_v_cache: jax.Array,
    A_wq: jax.Array,
    A_wo: jax.Array,
    B_x: jax.Array,
    B_c_kv: jax.Array,
    B_w_q: jax.Array,
    B_w_uk: jax.Array,
    B_w_uv: jax.Array,
    B_w_o: jax.Array,
):
    B, H, S, Dh = A_k_cache.shape
    M = A_x.shape[-1]
    Dc = B_c_kv.shape[-1]
    assert (B, H, S, Dh, M, Dc) == (4, 32, 4096, 128, 576, 512)
    bf16, f32 = jnp.bfloat16, jnp.float32
    n_m, n_c, n_lc, n_ck = M // _SEG, Dc // _SEG, H * Dh // _LC, S // _CK

    out = pl.pallas_call(
        _make_kernel(B, H, S, Dh, M, Dc),
        in_specs=[pl.BlockSpec(memory_space=pl.ANY)] * 11,
        out_specs=pl.BlockSpec(memory_space=pltpu.VMEM),
        out_shape=jax.ShapeDtypeStruct((B, 2 * M), A_x.dtype),
        scratch_shapes=[
            pltpu.VMEM((B, M), bf16),
            pltpu.VMEM((B, M), bf16),
            pltpu.VMEM((_NBUF, _G, _KC, Dh), bf16),
            pltpu.VMEM((_NBUF, _G, _KC, Dh), bf16),
            pltpu.VMEM((n_lc, n_m, _SEG, _LC), bf16),
            pltpu.VMEM((n_lc, n_m, _SEG, _LC), bf16),
            pltpu.VMEM((n_ck, B, n_ck, _CK // n_ck, Dc), bf16),
            pltpu.VMEM((n_m, _SEG * H, Dh), bf16),
            pltpu.VMEM((n_c, _SEG * H, Dh), bf16),
            pltpu.VMEM((n_c, _SEG * H, Dh), bf16),
            pltpu.VMEM((n_lc, H * M // n_lc, Dh), bf16),
            pltpu.VMEM((n_m, 8, _SEG), f32),
            pltpu.VMEM((H * 8, Dh), f32),
            pltpu.VMEM((B * H, Dh), f32),
            pltpu.VMEM((Dc // 128, H * 8, 128), f32),
            pltpu.VMEM((B, H, Dc), f32),
            pltpu.VMEM((B, H, 1), f32),
            pltpu.VMEM((B, H, 1), f32),
            pltpu.VMEM((B, H, Dc), f32),
        ],
        compiler_params=pltpu.CompilerParams(
            vmem_limit_bytes=80 * 1024 * 1024),
    )(
        A_x.reshape(B, M),
        B_x.reshape(B, M),
        A_k_cache.reshape(B * H // _G, _G, S, Dh),
        A_v_cache.reshape(B * H // _G, _G, S, Dh),
        A_wq.reshape(n_m, _SEG, H * Dh),
        A_wo.T.reshape(n_m, _SEG, H * Dh),
        B_c_kv.reshape(B, n_ck, _CK, Dc),
        B_w_q.reshape(n_m, _SEG * H, Dh),
        B_w_uk.reshape(n_c, _SEG * H, Dh),
        B_w_uv.reshape(n_c, _SEG * H, Dh),
        B_w_o.transpose(0, 2, 1).reshape(n_lc, H * M // n_lc, Dh),
    )
    return out.reshape(B, 1, 2 * M)
```

```python
import jax
import jax.numpy as jnp
import numpy as np
from jax import lax
import jax.experimental.pallas as pl
import jax.experimental.pallas.tpu as pltpu

_NT = (((1,), (1,)), ((), ()))
_NN = (((1,), (0,)), ((), ()))
_LOWEST = float(np.finfo(np.float32).min)

_G = 8
_KC = 512
_NBUF = 4
_SEG = 64
_LC = 512
_NCK = 4


def _dot(a, b, dims):
    return lax.dot_general(a, b, dims, preferred_element_type=jnp.float32)


def _ds(index, size):
    return pl.ds(pl.multiple_of(index * size, size), size)


def _loop(lo, count, body):
    lax.fori_loop(lo, lo + count, lambda i, carry: (body(i), carry)[1], 0)


def _share(n, parts, total, body):
    lo = lax.div(n * total, parts)
    _loop(lo, lax.div((n + 1) * total, parts) - lo, body)


def _wait(buf, sem):
    pltpu.make_async_copy(buf, buf, sem).wait()


def _halves(n):
    return enumerate((pl.ds(0, n // 2), pl.ds(n // 2, n - n // 2)))


def _split_heads(w, words_ref, n_heads):
    rows = w.shape[0] // n_heads
    words_ref[pl.ds(0, w.shape[0] // 2), :] = pltpu.bitcast(w, jnp.uint32)
    for j in range(n_heads // 2):
        words = words_ref[pl.ds(j, rows, stride=n_heads // 2), :]
        for half in (words << 16, (words >> 16) << 16):
            yield pltpu.bitcast(half, jnp.float32).astype(jnp.bfloat16)


def _softmax_step(state, s, pv):
    m, l, acc = state
    m_new = jnp.maximum(m, jnp.max(s, axis=-1, keepdims=True))
    alpha = jnp.exp(m - m_new)
    p = jnp.exp(s - m_new)
    l = alpha * l + jnp.sum(p, axis=-1, keepdims=True)
    acc = alpha * acc + pv(p.astype(jnp.bfloat16))
    return m_new, l, acc


def _make_kernel(B, H, S, Dh, M, Dc):
    bf16, f32 = jnp.bfloat16, jnp.float32
    scale = Dh ** -0.5
    n_m = M // _SEG
    n_cc = Dc // 128
    n_lc = H * Dh // _LC
    h_lc = _LC // Dh
    n_kc = S // _KC
    n_blocks = B * H // _G * n_kc
    kv_steps = _KC // 64
    ckv_steps = S // _NCK // _NCK // 16

    def body(xa_hbm, xb_hbm, k_hbm, v_hbm, awq_hbm, awo_hbm, ckv_hbm, bwq_hbm,
             wuk_hbm, wuv_hbm, bwo_hbm, out_ref,
             xa_buf, xb_buf, kv, awq, awo, ckv, bwq, wuk, wuv, bwo, words, xb_seg,
             by_head, by_batch, lat_head, lat_batch, lat_m, lat_l, lat_acc,
             kv_sem, awo_sem, ckv_sem, sem):
        xa_sem, xb_sem, bwq_sem, wuk_sem, awq_sem, wuv_sem, bwo_sem = (
            sem.at[n] for n in range(7))

        def tall_piece(src, dst, dma_sem):
            def piece(t):
                rows = _ds(t, 32)
                for priority, streams in _halves(src.shape[0]):
                    pltpu.make_async_copy(src.at[streams, rows], dst.at[streams, rows],
                                          dma_sem).start(priority=priority)
            return piece

        def wide_piece(src, dst, dma_sems, r, lc):
            rows = _ds(r, 8)
            for priority, streams in _halves(n_m):
                pltpu.make_async_copy(src.at[streams, rows, _ds(lc, _LC)],
                                      dst.at[lc, streams, rows],
                                      dma_sems[priority]).start(priority=priority)

        def awq_piece(t):
            wide_piece(awq_hbm, awq, (awq_sem, awq_sem), lax.div(t, n_lc), lax.rem(t, n_lc))

        def awo_piece(t):
            lc = lax.div(t, _SEG // 8)
            wide_piece(awo_hbm, awo, (awo_sem.at[2 * lc], awo_sem.at[2 * lc + 1]),
                       lax.rem(t, _SEG // 8), lc)

        def ckv_piece(t):
            chunk, rows = lax.div(t, ckv_steps), _ds(lax.rem(t, ckv_steps), 16)
            for b in range(B // 2):
                for s in range(0, _NCK, 2):
                    for priority, batch in enumerate((b, b + B // 2)):
                        pltpu.make_async_copy(ckv_hbm.at[batch, pl.ds(s, 2), _ds(t, 16)],
                                              ckv.at[chunk, batch, pl.ds(s, 2), rows],
                                              ckv_sem.at[chunk]).start(priority=priority)

        def kv_piece(t):
            slot = lax.rem(lax.div(t, kv_steps), _NBUF)
            group = lax.div(t, kv_steps * n_kc)
            src_rows = _ds(lax.rem(t, kv_steps * n_kc), 64)
            dst_rows = _ds(lax.rem(t, kv_steps), 64)
            for s in range(0, _G, 2):
                for priority, src in enumerate((k_hbm, v_hbm)):
                    pltpu.make_async_copy(src.at[group, pl.ds(s, 2), src_rows],
                                          kv.at[slot, priority, pl.ds(s, 2), dst_rows],
                                          kv_sem.at[slot]).start(priority=priority)

        wuv_piece = tall_piece(wuv_hbm, wuv, wuv_sem)
        bwo_piece = tall_piece(bwo_hbm, bwo, bwo_sem)

        _loop(0, 64, tall_piece(bwq_hbm, bwq, bwq_sem))
        x_copies = (pltpu.make_async_copy(xa_hbm, xa_buf, xa_sem),
                    pltpu.make_async_copy(xb_hbm, xb_buf, xb_sem))
        for c in x_copies:
            c.start()
        _loop(0, 64, tall_piece(wuk_hbm, wuk, wuk_sem))
        for c in x_copies:
            c.wait()

        def pad8(x_ref):
            return jnp.concatenate([x_ref[...].astype(f32), jnp.zeros((8 - B, M), f32)], axis=0)

        xb = pad8(xb_buf)
        for seg in range(n_m):
            xb_seg[seg] = xb[:, seg * _SEG:(seg + 1) * _SEG]
        by_head[...] = jnp.zeros(by_head.shape, f32)
        _wait(bwq, bwq_sem)

        def query_b(seg):
            x = xb_seg[seg].astype(bf16)
            for h, w in enumerate(_split_heads(bwq[seg], words, H)):
                by_head[pl.ds(h * 8, 8), :] += _dot(x, w, _NN)
            _loop(seg * 2, 2, ckv_piece)

        _loop(0, n_m, query_b)

        def latent_tiles(w_ref, cc):
            return _split_heads(w_ref[_ds(cc, 128 // _SEG)].reshape(128 * H, Dh), words, H)

        _wait(wuk, wuk_sem)

        def latent_query(cc):
            for h, w in enumerate(latent_tiles(wuk, cc)):
                rows = pl.ds(h * 8, 8)
                lat_head[cc, rows, :] = _dot(by_head[rows, :].astype(bf16), w, _NT)
            _loop(18 + cc * 4, 4, ckv_piece)

        _loop(0, n_cc, latent_query)

        for b in range(B):
            for cc in range(n_cc):
                lat_batch[b, :, cc * 128:(cc + 1) * 128] = lat_head[cc, pl.ds(b, H, stride=8), :]

        lat_m[...] = jnp.full(lat_m.shape, _LOWEST, f32)
        lat_l[...] = jnp.zeros(lat_l.shape, f32)
        lat_acc[...] = jnp.zeros(lat_acc.shape, f32)

        def latent_attention(i):
            chunk, b = lax.div(i, B), lax.rem(i, B)

            @pl.when(b == 0)
            def _():
                _wait(ckv.at[chunk], ckv_sem.at[chunk])

            cache = ckv[chunk, b].reshape(S // _NCK, Dc)
            s = _dot(lat_batch[b].astype(bf16), cache, _NT) * scale
            lat_m[b], lat_l[b], lat_acc[b] = _softmax_step(
                (lat_m[b], lat_l[b], lat_acc[b]), s, lambda p: _dot(p, cache, _NN))

            @pl.when(i < 6)
            def _():
                _loop(34 + i * 5, 5, ckv_piece)

            @pl.when(i >= 6)
            def _():
                for piece, total in ((wuv_piece, 64), (awq_piece, 64), (bwo_piece, 72)):
                    _share(i - 6, B * _NCK - 6, total, piece)

        _loop(0, B * _NCK, latent_attention)

        for b in range(B):
            ctx = lat_acc[b] / lat_l[b]
            for cc in range(n_cc):
                lat_head[cc, pl.ds(b, H, stride=8), :] = ctx[:, cc * 128:(cc + 1) * 128]

        _loop(0, 8, kv_piece)
        by_head[...] = jnp.zeros(by_head.shape, f32)
        _wait(wuv, wuv_sem)

        def context_b(cc):
            for h, w in enumerate(latent_tiles(wuv, cc)):
                rows = pl.ds(h * 8, 8)
                by_head[rows, :] += _dot(lat_head[cc, rows, :].astype(bf16), w, _NN)
            _loop(8 + cc * 4, 4, kv_piece)

        _loop(0, n_cc, context_b)
        _wait(bwo, bwo_sem)
        _wait(awq, awq_sem)
        xa = pad8(xa_buf).astype(bf16)

        def project_b_query_a(lc, out_b):
            q = _dot(xa, awq[lc].reshape(M, _LC), _NN)
            for t in range(h_lc):
                rows = _ds(lc * h_lc + t, 8)
                out_b += _dot(by_head[rows, :].astype(bf16), bwo[lc, pl.ds(t * M, M), :], _NT)
                by_head[rows, :] = q[:, t * Dh:(t + 1) * Dh]
            kv_piece(24 + lc)
            return out_b

        out_b = lax.fori_loop(0, n_lc, project_b_query_a, jnp.zeros((8, M), f32))
        out_ref[:, M:] = out_b[:B].astype(out_ref.dtype)

        for b in range(B):
            by_batch[pl.ds(b * H, H), :] = by_head[pl.ds(b, H, stride=8), :]

        def diagonal(parts):
            row = lax.broadcasted_iota(jnp.int32, parts[0].shape, 0)
            out = parts[0]
            for j in range(1, _G):
                out = jnp.where(row == j, parts[j], out)
            return out

        def attention(i, state):
            slot = lax.rem(i, _NBUF)
            heads, chunk = _ds(lax.div(i, n_kc), _G), lax.rem(i, n_kc)
            _wait(kv.at[slot], kv_sem.at[slot])
            q = by_batch[heads, :].astype(bf16)
            s = diagonal([_dot(q, kv[slot, 0, j], _NT) for j in range(_G)]) * scale
            state = tuple(jnp.where(chunk == 0, fill, x)
                          for fill, x in zip((_LOWEST, 0.0, 0.0), state))
            state = _softmax_step(
                state, s,
                lambda p: diagonal([_dot(p, kv[slot, 1, j], _NN) for j in range(_G)]))

            @pl.when(chunk == n_kc - 1)
            def _():
                by_batch[heads, :] = state[2] / state[1]

            @pl.when(i + _NBUF < n_blocks)
            def _():
                _loop((i + _NBUF) * kv_steps, kv_steps, kv_piece)

            @pl.when(i + _NBUF >= n_blocks)
            def _():
                _share(i + _NBUF - n_blocks, _NBUF, 64, awo_piece)

            return state

        lax.fori_loop(0, n_blocks, attention,
                      tuple(jnp.zeros((_G, n), f32) for n in (1, 1, Dh)))

        for b in range(B):
            by_head[pl.ds(b, H, stride=8), :] = by_batch[pl.ds(b * H, H), :]

        def project_a(lc, out_a):
            o = jnp.concatenate([by_head[_ds(lc * h_lc + t, 8), :] for t in range(h_lc)], axis=1)
            parts = []
            for priority, streams in _halves(n_m):
                _wait(awo.at[lc, streams], awo_sem.at[2 * lc + priority])
                parts.append(_dot(o.astype(bf16), awo[lc, streams].reshape(-1, _LC), _NT))
            return out_a + jnp.concatenate(parts, axis=1)

        out_a = lax.fori_loop(0, n_lc, project_a, jnp.zeros((8, M), f32))
        out_ref[:, :M] = out_a[:B].astype(out_ref.dtype)

    def kernel(*refs):
        pl.run_scoped(lambda *sems: body(*refs, *sems),
                      *(pltpu.SemaphoreType.DMA((n,)) for n in (_NBUF, 2 * n_lc, _NCK, 7)))

    return kernel


@jax.jit
def pallas_concat_heads__mha_block_cached__compressed_kv_cla__decode_kernel(
    A_x: jax.Array,
    A_k_cache: jax.Array,
    A_v_cache: jax.Array,
    A_wq: jax.Array,
    A_wo: jax.Array,
    B_x: jax.Array,
    B_c_kv: jax.Array,
    B_w_q: jax.Array,
    B_w_uk: jax.Array,
    B_w_uv: jax.Array,
    B_w_o: jax.Array,
):
    B, H, S, Dh = A_k_cache.shape
    M = A_x.shape[-1]
    Dc = B_c_kv.shape[-1]
    assert (B, H, S, Dh, M, Dc) == (4, 32, 4096, 128, 576, 512)
    bf16, f32 = jnp.bfloat16, jnp.float32
    n_m, n_c, n_lc = M // _SEG, Dc // _SEG, H * Dh // _LC

    out = pl.pallas_call(
        _make_kernel(B, H, S, Dh, M, Dc),
        in_specs=[pl.BlockSpec(memory_space=pl.ANY)] * 11,
        out_specs=pl.BlockSpec(memory_space=pltpu.VMEM),
        out_shape=jax.ShapeDtypeStruct((B, 2 * M), A_x.dtype),
        scratch_shapes=[
            pltpu.VMEM((B, M), bf16),
            pltpu.VMEM((B, M), bf16),
            pltpu.VMEM((_NBUF, 2, _G, _KC, Dh), bf16),
            pltpu.VMEM((n_lc, n_m, _SEG, _LC), bf16),
            pltpu.VMEM((n_lc, n_m, _SEG, _LC), bf16),
            pltpu.VMEM((_NCK, B, _NCK, S // _NCK // _NCK, Dc), bf16),
            pltpu.VMEM((n_m, _SEG * H, Dh), bf16),
            pltpu.VMEM((n_c, _SEG * H, Dh), bf16),
            pltpu.VMEM((n_c, _SEG * H, Dh), bf16),
            pltpu.VMEM((n_lc, H * M // n_lc, Dh), bf16),
            pltpu.VMEM((128 * H // 2, Dh), jnp.uint32),
            pltpu.VMEM((n_m, 8, _SEG), f32),
            pltpu.VMEM((H * 8, Dh), f32),
            pltpu.VMEM((B * H, Dh), f32),
            pltpu.VMEM((Dc // 128, H * 8, 128), f32),
            pltpu.VMEM((B, H, Dc), f32),
            pltpu.VMEM((B, H, 1), f32),
            pltpu.VMEM((B, H, 1), f32),
            pltpu.VMEM((B, H, Dc), f32),
        ],
        compiler_params=pltpu.CompilerParams(vmem_limit_bytes=80 * 1024 * 1024),
    )(
        A_x.reshape(B, M),
        B_x.reshape(B, M),
        A_k_cache.reshape(B * H // _G, _G, S, Dh),
        A_v_cache.reshape(B * H // _G, _G, S, Dh),
        A_wq.reshape(n_m, _SEG, H * Dh),
        A_wo.T.reshape(n_m, _SEG, H * Dh),
        B_c_kv.reshape(B, _NCK, S // _NCK, Dc),
        B_w_q.reshape(n_m, _SEG * H, Dh),
        B_w_uk.reshape(n_c, _SEG * H, Dh),
        B_w_uv.reshape(n_c, _SEG * H, Dh),
        B_w_o.transpose(0, 2, 1).reshape(n_lc, H * M // n_lc, Dh),
    )
    return out.reshape(B, 1, 2 * M)
```
